```python
import jax
import jax.numpy as jnp

def _softmax(x, axis=-1):
    return jax.nn.softmax(x, axis=axis)

def _gelu(x):
    return jax.nn.gelu(x, approximate=True)

def _silu(x):
    return jax.nn.silu(x)

def _sigmoid(x):
    return jax.nn.sigmoid(x)

def _layernorm(x, axis=-1, eps=1e-05):
    m = jnp.mean(x, axis=axis, keepdims=True)
    v = jnp.var(x, axis=axis, keepdims=True)
    return (x - m) / jnp.sqrt(v + eps)

def _scatter_add(tgt, idx, src, axis=0):
    return tgt.at[idx].add(src)

def _segment_sum(src, seg, n):
    return jax.ops.segment_sum(src, seg, n)

class _Rng:

    def __init__(self, key):
        self._k = key

    def _next(self):
        self._k, sub = jax.random.split(self._k)
        return sub

    def normal(self, shape):
        return jax.random.normal(self._next(), shape, dtype=jnp.bfloat16)

    def randint(self, lo, hi, shape):
        return jax.random.randint(self._next(), shape, lo, hi, dtype=jnp.int32)

    def uniform(self, shape, lo=0.0, hi=1.0):
        return jax.random.uniform(self._next(), shape, jnp.bfloat16, lo, hi)

    def permutation(self, n):
        return jax.random.permutation(self._next(), n)
kernel_name = 'interleave_layers__linear_kernel_hedgehog__mixer_gmlp__prompt'

def _fwd_setup_inputs():
    _rng = _Rng(jax.random.key(int.from_bytes(__import__("os").urandom(4), "little")))
    _w = lambda a: (lambda t: t.astype(jnp.bfloat16) if jnp.issubdtype(t.dtype, jnp.floating) else t)(jnp.asarray(a))

    def _A_setup():
        B, S, D, H = (1, 2048, 640, 32)
        Dh = D // H
        return {'x': _w((lambda *s: _rng.normal(s) * 0.05)(B, S, D)), 'wqkv': _w((lambda *s: _rng.normal(s) * 0.05)(D, 3 * D)), 'w_phi': _w((lambda *s: _rng.normal(s) * 0.05)(H, Dh, Dh) * Dh ** (-0.5)), 'wo': _w((lambda *s: _rng.normal(s) * 0.05)(D, D))}
    _A_in = _A_setup()

    def _B_setup():
        B, S, D, F = (1, 2048, 640, 1536)
        Fh = F // 2
        return {'x': _w((lambda *s: _rng.normal(s) * 0.05)(B, S, D)), 'w_in': _w((lambda *s: _rng.normal(s) * 0.05)(D, 2 * Fh)), 'w_sp': _w(0.01 * (lambda *s: _rng.normal(s) * 0.05)(S, S)), 'b_sp': _w(1.0 + 0.01 * (lambda *s: _rng.normal(s) * 0.05)(S)), 'w_out': _w((lambda *s: _rng.normal(s) * 0.05)(Fh, D))}
    _B_in = _B_setup()
    return {'A_x': _A_in['x'], 'A_wqkv': _A_in['wqkv'], 'A_w_phi': _A_in['w_phi'], 'A_wo': _A_in['wo'], 'B_x': _B_in['x'], 'B_w_in': _B_in['w_in'], 'B_w_sp': _B_in['w_sp'], 'B_b_sp': _B_in['b_sp'], 'B_w_out': _B_in['w_out']}

def _fwd_reference(A_x, A_wqkv, A_w_phi, A_wo, B_x, B_w_in, B_w_sp, B_b_sp, B_w_out):

    def _A_ref(x, wqkv, w_phi, wo):
        B, S, D = x.shape
        H = 32
        Dh = D // H
        qkv = (lambda x, *d: x.transpose(*d))((x @ wqkv).reshape(B, S, 3, H, Dh), 2, 0, 3, 1, 4)
        q, k, v = (qkv[0], qkv[1], qkv[2])
        pq = jnp.einsum('bhsd,hdf->bhsf', q, w_phi)
        pk = jnp.einsum('bhsd,hdf->bhsf', k, w_phi)
        phi_q = jnp.concatenate([_softmax(pq, axis=-1), _softmax(-pq, axis=-1)], axis=-1)
        phi_k = jnp.concatenate([_softmax(pk, axis=-1), _softmax(-pk, axis=-1)], axis=-1)
        kv = jnp.einsum('bhsf,bhsd->bhfd', phi_k, v)
        z = jnp.einsum('bhsf->bhf', phi_k)
        num = jnp.einsum('bhqf,bhfd->bhqd', phi_q, kv)
        den = jnp.einsum('bhqf,bhf->bhq', phi_q, z)[..., None] + 1e-06
        o = num / den
        return (lambda x, *d: x.transpose(*d))(o, 0, 2, 1, 3).reshape(B, S, D) @ wo

    def _B_ref(x, w_in, w_sp, b_sp, w_out):
        B, S, D = x.shape
        F = w_in.shape[-1]
        Fh = F // 2
        z = _gelu(jnp.einsum('bsd,df->bsf', x, w_in))
        z1 = z[..., :Fh].copy()
        z2 = _layernorm(z[..., Fh:], axis=-1)
        g = jnp.einsum('ts,bsf->btf', w_sp, z2) + b_sp[None, :, None]
        return jnp.einsum('bsf,fd->bsd', z1 * g, w_out)
    x = A_x
    x = x + _A_ref(_layernorm(x, axis=-1), A_wqkv, A_w_phi, A_wo)
    x = x + _B_ref(_layernorm(x, axis=-1), B_w_in, B_w_sp, B_b_sp, B_w_out)
    x = x + _A_ref(_layernorm(x, axis=-1), A_wqkv, A_w_phi, A_wo)
    x = x + _B_ref(_layernorm(x, axis=-1), B_w_in, B_w_sp, B_b_sp, B_w_out)
    return x

def setup_inputs():
    _inp = _fwd_setup_inputs()
    _gk = jax.random.fold_in(jax.random.key(int.from_bytes(__import__("os").urandom(4), "little")), 2 ** 31 - 1)
    _shapes = [[1, 2048, 640]]
    _dtypes = ['bfloat16']
    _gks = jax.random.split(_gk, len(_shapes))
    _gs = [jax.random.normal(k, s, dtype=jnp.dtype(d)) * 0.05 for k, s, d in zip(_gks, _shapes, _dtypes)]
    _inp['grad_out'] = _gs[0]
    return _inp

def reference(A_x, A_wqkv, A_w_phi, A_wo, B_w_in, B_w_sp, B_b_sp, B_w_out, B_x, grad_out):
    _const = dict(B_x=B_x)

    def _f(*_d):
        return _fwd_reference(**{'A_x': _d[0], 'A_wqkv': _d[1], 'A_w_phi': _d[2], 'A_wo': _d[3], 'B_w_in': _d[4], 'B_w_sp': _d[5], 'B_b_sp': _d[6], 'B_w_out': _d[7], **_const})
    _out, _vjp = jax.vjp(_f, A_x, A_wqkv, A_w_phi, A_wo, B_w_in, B_w_sp, B_b_sp, B_w_out)
    _grads = _vjp(grad_out)
    _out0 = jnp.asarray(_out)
    return (_out0, *[jnp.asarray(_g) for _g in _grads])
```

```python
import jax
import jax.numpy as jnp
from jax import lax
import jax.experimental.pallas as pl
import jax.experimental.pallas.tpu as pltpu

S, D, H, DH, F, FH = 2048, 640, 32, 20, 1536, 768
NG = 4
GR = 160
GA = 176
TN = 256
NB = S // TN
TW = 256
F32, BF16 = jnp.float32, jnp.bfloat16

_NN = (((1,), (0,)), ((), ()))
_NT = (((1,), (1,)), ((), ()))
_TN = (((0,), (0,)), ((), ()))


def _nn(a, b):
    return lax.dot_general(a, b, _NN, preferred_element_type=F32)


def _nt(a, b):
    return lax.dot_general(a, b, _NT, preferred_element_type=F32)


def _tn(a, b):
    return lax.dot_general(a, b, _TN, preferred_element_type=F32)


def _iota(shape, d):
    return lax.broadcasted_iota(jnp.int32, shape, d)


def _ln_fwd(x):
    m = jnp.mean(x, axis=0, keepdims=True)
    xc = x - m
    r = lax.rsqrt(jnp.mean(xc * xc, axis=0, keepdims=True) + 1e-5)
    return xc * r, r


def _ln_bwd(dy, y, r):
    m1 = jnp.mean(dy, axis=0, keepdims=True)
    m2 = jnp.mean(dy * y, axis=0, keepdims=True)
    return r * (dy - m1 - y * m2)


def _gelu_and_grad(u):
    c = 0.7978845608028654
    u2 = u * u
    t = jnp.tanh(u * (c + (c * 0.044715) * u2))
    h = 0.5 * t + 0.5
    return u * h, h + (0.5 * u) * (1.0 - t * t) * (c + (3 * c * 0.044715) * u2)


def _phi(t):
    n = t.shape[-1]
    t = t.reshape(DH, 8, n)
    ep = jnp.exp(t - jnp.max(t, axis=0, keepdims=True))
    en = jnp.exp(jnp.min(t, axis=0, keepdims=True) - t)
    p = ep * (1.0 / jnp.sum(ep, axis=0, keepdims=True))
    q = en * (1.0 / jnp.sum(en, axis=0, keepdims=True))
    return p.reshape(GR, n), q.reshape(GR, n)


def _phi_bwd(dphi, phi):
    n = dphi.shape[-1]
    p = phi[:GR].astype(F32).reshape(DH, 8, n)
    q = phi[GR:].astype(F32).reshape(DH, 8, n)
    dp = dphi[:GR].reshape(DH, 8, n) * p
    dq = dphi[GR:].reshape(DH, 8, n) * q
    dt = (dp - p * jnp.sum(dp, axis=0, keepdims=True)) - (dq - q * jnp.sum(dq, axis=0, keepdims=True))
    return dt.reshape(GR, n)


def _kernel(
    x_h, wqkv_h, wphi_h, wo_h, win_h, wsp_h, bsp_h, wout_h, g_h,
    out_h, dx_h, dwqkv_h, dwphi_h, dwo_h, dwin_h, dwsp_h, dbsp_h, dwout_h,
    io, wqkv, wphi, wo, win, wsp, bsp, wout,
    wqkT, wpT, wp, woT, wop, winT, woutT, mT, mN, wphi2,
    xs, lnA, rA, phq, phk, va, oo, idn, kvT, kvN,
    lnB, rB, z1s, gp1, gp2, z2n, r2, gs,
    kacc, dkvT, dkvN, dwT, dwo_a, dwin_a, dwout_a, dbs, wsel, dwphi_s, dbo,
    sem,
):
    def cp(src, dst, i):
        return pltpu.make_async_copy(src, dst, sem.at[i])

    loads = [cp(x_h, io, 0), cp(wqkv_h, wqkv, 1), cp(wphi_h, wphi, 2), cp(wo_h, wo, 3),
             cp(win_h, win, 4), cp(wout_h, wout, 5), cp(bsp_h, bsp, 6), cp(wsp_h, wsp, 7)]
    for c in loads:
        c.start()

    def blk(j):
        return pl.ds(pl.multiple_of(j * TN, TN), TN)

    def loop(body):
        def f(j, c):
            body(j, blk(j))
            return c
        lax.fori_loop(0, NB, f, 0)

    ci = _iota((GR, GR), 1)
    ri = _iota((GR, GR), 0)
    perm = (((ri & 7) * DH + (ri >> 3)) == ci).astype(BF16)
    hmaskT = lax.div(ci, DH) == (ri & 7)
    hmaskN = lax.div(ri, DH) == (ci & 7)
    eT = ((_iota((GR, 128), 0) >> 3) == _iota((GR, 128), 1)).astype(BF16)

    aug = (_iota((GA - GR, S), 0) < 8).astype(BF16)
    for l in range(2):
        for g in range(NG):
            va[l, g * GA + GR:(g + 1) * GA, :] = aug

    loads[2].wait()
    wphi2[...] = jnp.zeros_like(wphi2)
    for h in range(H):
        wphi2[h * DH:(h + 1) * DH, 0:DH] = wphi[h].astype(F32)
    for g in range(NG):
        w2 = wphi2[g * GR:(g + 1) * GR, :].astype(BF16)
        mT[g] = jnp.where(hmaskT, _nt(eT, w2), 0.0).astype(BF16)
        mN[g] = jnp.where(hmaskN, _nt(w2, eT), 0.0).astype(BF16)
    loads[1].wait()
    for part in range(3):
        wt = wqkv[:, part * D:(part + 1) * D].astype(F32).T.astype(BF16)
        if part < 2:
            wqkT[part * D:(part + 1) * D, :] = wt
        for g in range(NG):
            m = mT[g] if part < 2 else perm
            wpT[part * D + g * GR:part * D + (g + 1) * GR, :] = _nn(m, wt[g * GR:(g + 1) * GR]).astype(BF16)
        wp[:, part * D:(part + 1) * D] = wpT[part * D:(part + 1) * D, :].astype(F32).T.astype(BF16)
    loads[3].wait()
    for g in range(NG):
        wop[g * GR:(g + 1) * GR, :] = _nn(perm, wo[g * GR:(g + 1) * GR, :]).astype(BF16)
    woT[...] = wop[...].astype(F32).T.astype(BF16)
    loads[0].wait()

    def a_fwd1(l, b, x):
        y, r = _ln_fwd(x)
        rA[l, :, b] = r
        yb = y.astype(BF16)
        lnA[l, :, b] = yb
        for part, dst in ((0, phq), (1, phk)):
            t = _nn(wpT[part * D:(part + 1) * D, :], yb)
            for g in range(NG):
                p, q = _phi(t[g * GR:(g + 1) * GR])
                dst[l, 2 * g * GR:(2 * g + 1) * GR, b] = p.astype(BF16)
                dst[l, (2 * g + 1) * GR:(2 * g + 2) * GR, b] = q.astype(BF16)
        v = _nn(wpT[2 * D:3 * D, :], yb).astype(BF16)
        for g in range(NG):
            va[l, g * GA:g * GA + GR, b] = v[g * GR:(g + 1) * GR]
            kacc[g] += _nt(va[l, g * GA:(g + 1) * GA, b], phk[l, 2 * g * GR:(2 * g + 2) * GR, b])

    kmask = (_iota((GA, 2 * GR), 0) & 7) == (_iota((GA, 2 * GR), 1) & 7)

    def kv_zero():
        kacc[...] = jnp.zeros_like(kacc)

    def kv_done(outT, outN):
        for g in range(NG):
            k = jnp.where(kmask, kacc[g], 0.0)
            outT[g] = k.astype(BF16)
            outN[g] = k.T.astype(BF16)

    def a_fwd2(l, b):
        for g in range(NG):
            nd = _nn(kvT[l * NG + g], phq[l, 2 * g * GR:(2 * g + 2) * GR, b])
            inv = 1.0 / (nd[GR:GR + 8] + 1e-6)
            idn[l, g * 8:(g + 1) * 8, b] = inv
            o = nd[:GR].reshape(DH, 8, TN) * inv[None]
            oo[l, g * GR:(g + 1) * GR, b] = o.reshape(GR, TN).astype(BF16)
        x = xs[:, b] + _nn(woT[...], oo[l, :, b])
        xs[:, b] = x
        return x

    def b_fwd1(l, b, x):
        y, r = _ln_fwd(x)
        rB[l, :, b] = r
        yb = y.astype(BF16)
        lnB[l, :, b] = yb
        z, gp = _gelu_and_grad(_nn(winT[0:FH, :], yb))
        z1s[l * FH:(l + 1) * FH, b] = z.astype(BF16)
        gp1[l, :, b] = gp.astype(BF16)
        z, gp = _gelu_and_grad(_nn(winT[FH:F, :], yb))
        gp2[l, :, b] = gp.astype(BF16)
        zn, r = _ln_fwd(z)
        r2[l, :, b] = r
        z2n[l * FH:(l + 1) * FH, b] = zn.astype(BF16)

    def b_fwd2(l, b):
        g = _nt(z2n[l * FH:(l + 1) * FH, :], wsp[b, :]) + bsp[:, b].astype(F32)
        z1 = z1s[l * FH:(l + 1) * FH, b].astype(F32)
        p = (z1 * g).astype(BF16)
        x = xs[:, b] + _nn(woutT[...], p)
        return x, g, z1, p

    def b_bwd1(l, b, dx, g, z1, p, first):
        dob = dx.astype(BF16)
        dp = _nn(wout[...], dob)
        dwout_a[...] += _nt(p, dob)
        gp1[l, :, b] = (dp * g * gp1[l, :, b].astype(F32)).astype(BF16)
        dg = dp * z1
        cs = jnp.sum(dg, axis=0, keepdims=True)
        if first:
            dbs[:, b] = cs
        else:
            dbs[:, b] += cs
        z1s[l * FH:(l + 1) * FH, b] = dg.astype(BF16)

    def b_bwd2(l, b):
        dzn = _nn(z1s[l * FH:(l + 1) * FH, :], wsp[:, b])
        dz = _ln_bwd(dzn, z2n[l * FH:(l + 1) * FH, b].astype(F32), r2[l, :, b])
        du2 = (dz * gp2[l, :, b].astype(F32)).astype(BF16)
        du1 = gp1[l, :, b]
        y = lnB[l, :, b]
        dwin_a[:, 0:FH] += _nt(y, du1)
        dwin_a[:, FH:F] += _nt(y, du2)
        dy = _nn(win[:, 0:FH], du1) + _nn(win[:, FH:F], du2)
        dx = xs[:, b] + _ln_bwd(dy, y.astype(F32), rB[l, :, b])
        xs[:, b] = dx
        return dx

    def a_bwd1(l, b, dx):
        dob = dx.astype(BF16)
        do = _nn(wop[...], dob)
        ob = oo[l, :, b]
        dwo_a[...] += _nt(ob, dob)
        for g in range(NG):
            inv = idn[l, g * 8:(g + 1) * 8, b]
            dn = do[g * GR:(g + 1) * GR].reshape(DH, 8, TN) * inv[None]
            o = ob[g * GR:(g + 1) * GR].astype(F32).reshape(DH, 8, TN)
            dd = -jnp.sum(dn * o, axis=0)
            a = jnp.concatenate([dn.reshape(GR, TN), dd, jnp.zeros((8, TN), F32)], axis=0).astype(BF16)
            pq = phq[l, 2 * g * GR:(2 * g + 2) * GR, b]
            kacc[g] += _nt(a, pq)
            dphi = _nn(kvN[l * NG + g], a)
            dt = _phi_bwd(dphi, pq)
            oo[l, g * GR:(g + 1) * GR, b] = dt.astype(BF16)

    def a_bwd2(l, b):
        dks, dvs = [], []
        for g in range(NG):
            pk = phk[l, 2 * g * GR:(2 * g + 2) * GR, b]
            dphi = _nn(dkvN[g], va[l, g * GA:(g + 1) * GA, b])
            dks.append(_phi_bwd(dphi, pk).astype(BF16))
            dvs.append(_nn(dkvT[g, 0:GR, :], pk).astype(BF16))
        dp = jnp.concatenate([oo[l, :, b]] + dks + dvs, axis=0)
        y = lnA[l, :, b]
        dwT[...] += _nt(dp, y)
        dy = _nn(wp[...], dp)
        return xs[:, b] + _ln_bwd(dy, y.astype(F32), rA[l, :, b])

    def f1(j, b):
        x = io[b, :].astype(F32).T
        xs[:, b] = x
        a_fwd1(0, b, x)
    kv_zero()
    loop(f1)
    gload = cp(g_h, io, 0)
    gload.start()
    loads[4].wait()
    loads[5].wait()
    winT[...] = win[...].astype(F32).T.astype(BF16)
    woutT[...] = wout[...].astype(F32).T.astype(BF16)

    def f2(l):
        def body(j, b):
            b_fwd1(l, b, a_fwd2(l, b))
        return body

    kv_done(kvT.at[0:NG], kvN.at[0:NG])
    loop(f2(0))
    loads[6].wait()
    loads[7].wait()

    def f3(j, b):
        x, g, _, _ = b_fwd2(0, b)
        gs[:, b] = g.astype(BF16)
        xs[:, b] = x
        a_fwd1(1, b, x)
    kv_zero()
    loop(f3)
    kv_done(kvT.at[NG:2 * NG], kvN.at[NG:2 * NG])
    loop(f2(1))

    dwout_a[...] = jnp.zeros_like(dwout_a)
    dwin_a[...] = jnp.zeros_like(dwin_a)
    dwo_a[...] = jnp.zeros_like(dwo_a)
    dwT[...] = jnp.zeros_like(dwT)
    gload.wait()

    def f5(j, b):
        x, g, z1, p = b_fwd2(1, b)
        dx = io[b, :].astype(F32).T
        io[b, :] = x.T.astype(BF16)
        xs[:, b] = dx
        b_bwd1(1, b, dx, g, z1, p, True)
    loop(f5)
    ostore = cp(io, out_h, 0)
    ostore.start()

    def bx(l):
        def body(j, b):
            a_bwd1(l, b, b_bwd2(l, b))
        return body

    kv_zero()
    loop(bx(1))
    kv_done(dkvT, dkvN)

    def by(j, b):
        dx = a_bwd2(1, b)
        xs[:, b] = dx
        g = gs[:, b].astype(F32)
        z1 = z1s[0:FH, b].astype(F32)
        b_bwd1(0, b, dx, g, z1, (z1 * g).astype(BF16), False)
    loop(by)

    def wsp_copy(j, slot):
        return cp(wsel.at[slot], dwsp_h.at[pl.ds(pl.multiple_of(j * TW, TW), TW), :], 8 + slot)

    def bx0(j, b):
        for k in range(TN // TW):
            @pl.when(j >= 1)
            def _():
                wsp_copy(j, k).wait()
            tb = pl.ds(pl.multiple_of(j * TN + k * TW, TW), TW)
            wsel[k] = _tn(z1s[:, tb], z2n[...]).astype(BF16)
            wsp_copy(j * (TN // TW) + k, k).start()
        a_bwd1(0, b, b_bwd2(0, b))
    kv_zero()
    loop(bx0)
    for k in range(TN // TW):
        wsp_copy(0, k).wait()

    win[...] = dwin_a[...].astype(BF16)
    wout[...] = dwout_a[...].astype(BF16)
    dbo[...] = dbs[...].astype(BF16)
    permN = (((ci & 7) * DH + (ci >> 3)) == ri).astype(BF16)
    for g in range(NG):
        wo[g * GR:(g + 1) * GR, :] = _nn(permN, dwo_a[g * GR:(g + 1) * GR, :].astype(BF16)).astype(BF16)
    stores = [cp(win, dwin_h, 1), cp(wout, dwout_h, 2), cp(dbo, dbsp_h, 3), cp(wo, dwo_h, 4)]
    for c in stores:
        c.start()
    kv_done(dkvT, dkvN)
    ostore.wait()

    def bz(j, b):
        io[b, :] = a_bwd2(0, b).T.astype(BF16)
    loop(bz)
    xstore = cp(io, dx_h, 0)
    xstore.start()

    for part in range(3):
        for g in range(NG):
            rows = slice(part * D + g * GR, part * D + (g + 1) * GR)
            m = mN[g] if part < 2 else permN
            wpT[rows, :] = _nn(m, dwT[rows, :].astype(BF16)).astype(BF16)
        wqkv[:, part * D:(part + 1) * D] = wpT[part * D:(part + 1) * D, :].astype(F32).T.astype(BF16)
    qstore = cp(wqkv, dwqkv_h, 5)
    qstore.start()
    for g in range(NG):
        rq = slice(g * GR, (g + 1) * GR)
        rk = slice(D + g * GR, D + (g + 1) * GR)
        dm = _nt(wqkT[rq, :], dwT[rq, :].astype(BF16)) + _nt(wqkT[rk, :], dwT[rk, :].astype(BF16))
        dm = jnp.where(hmaskN, dm, 0.0).astype(BF16)
        wphi2[rq, :] = _nn(dm, eT)
    for h in range(H):
        dwphi_s[h] = wphi2[h * DH:(h + 1) * DH, 0:DH].astype(BF16)
    pstore = cp(dwphi_s, dwphi_h, 6)
    pstore.start()
    for c in stores + [xstore, qstore, pstore]:
        c.wait()


@jax.jit
def pallas_interleave_layers__linear_kernel_hedgehog__mixer_gmlp__prompt_kernel(
    A_x: jax.Array,
    A_wqkv: jax.Array,
    A_w_phi: jax.Array,
    A_wo: jax.Array,
    B_x: jax.Array,
    B_w_in: jax.Array,
    B_w_sp: jax.Array,
    B_b_sp: jax.Array,
    B_w_out: jax.Array,
    grad_out: jax.Array,
):
    del B_x
    sds = jax.ShapeDtypeStruct
    V = pltpu.VMEM
    scratch = [
        V((S, D), BF16), V((D, 3 * D), BF16), V((H, DH, DH), BF16), V((D, D), BF16),
        V((D, F), BF16), V((S, S), BF16), V((1, S), BF16), V((FH, D), BF16),
        V((2 * D, D), BF16), V((3 * D, D), BF16), V((D, 3 * D), BF16), V((D, D), BF16),
        V((D, D), BF16), V((F, D), BF16), V((D, FH), BF16),
        V((NG, GR, GR), BF16), V((NG, GR, GR), BF16), V((D, 128), F32),
        V((D, S), F32), V((2, D, S), BF16), V((2, 1, S), F32),
        V((2, 2 * D, S), BF16), V((2, 2 * D, S), BF16), V((2, NG * GA, S), BF16),
        V((2, D, S), BF16), V((2, H, S), F32),
        V((2 * NG, GA, 2 * GR), BF16), V((2 * NG, 2 * GR, GA), BF16),
        V((2, D, S), BF16), V((2, 1, S), F32), V((2 * FH, S), BF16), V((2, FH, S), BF16),
        V((2, FH, S), BF16), V((2 * FH, S), BF16), V((2, 1, S), F32), V((FH, S), BF16),
        V((NG, GA, 2 * GR), F32), V((NG, GA, 2 * GR), BF16), V((NG, 2 * GR, GA), BF16),
        V((3 * D, D), F32), V((D, D), F32), V((D, F), F32), V((FH, D), F32),
        V((1, S), F32), V((TN // TW, TW, S), BF16), V((H, DH, DH), BF16), V((1, S), BF16),
        pltpu.SemaphoreType.DMA((8 + TN // TW,)),
    ]
    out_shape = (
        sds((S, D), BF16), sds((S, D), BF16), sds((D, 3 * D), BF16), sds((H, DH, DH), BF16),
        sds((D, D), BF16), sds((D, F), BF16), sds((S, S), BF16), sds((1, S), BF16),
        sds((FH, D), BF16),
    )
    any_spec = pl.BlockSpec(memory_space=pl.ANY)
    out, dx, dwqkv, dwphi, dwo, dwin, dwsp, dbsp, dwout = pl.pallas_call(
        _kernel,
        out_shape=out_shape,
        in_specs=[any_spec] * 9,
        out_specs=(any_spec,) * 9,
        scratch_shapes=scratch,
        compiler_params=pltpu.CompilerParams(vmem_limit_bytes=128 * 2**20),
    )(A_x.reshape(S, D), A_wqkv, A_w_phi, A_wo, B_w_in, B_w_sp, B_b_sp.reshape(1, S),
      B_w_out, grad_out.reshape(S, D))
    return (out.reshape(1, S, D), dx.reshape(1, S, D), dwqkv, dwphi, dwo, dwin, dwsp,
            dbsp.reshape(S), dwout)
```
